```python
import os as _os
_os.environ.setdefault("JAX_PLATFORMS", "cpu")
import jax
import jax.numpy as jnp

def _softmax(x, axis=-1):
    return jax.nn.softmax(x, axis=axis)
def _gelu(x):
    return jax.nn.gelu(x, approximate=True)
def _silu(x):
    return jax.nn.silu(x)
def _sigmoid(x):
    return jax.nn.sigmoid(x)
def _layernorm(x, axis=-1, eps=1e-5):
    m = jnp.mean(x, axis=axis, keepdims=True)
    v = jnp.var(x, axis=axis, keepdims=True)
    return (x - m) / jnp.sqrt(v + eps)
def _scatter_add(tgt, idx, src, axis=0):
    return tgt.at[idx].add(src)
def _segment_sum(src, seg, n):
    return jax.ops.segment_sum(src, seg, n)
class _Rng:
    def __init__(self, key):
        self._k = key
    def _next(self):
        self._k, sub = jax.random.split(self._k)
        return sub
    def normal(self, shape):
        return jax.random.normal(self._next(), shape, dtype=jnp.bfloat16)
    def randint(self, lo, hi, shape):
        return jax.random.randint(self._next(), shape, lo, hi, dtype=jnp.int32)
    def uniform(self, shape, lo=0.0, hi=1.0):
        return jax.random.uniform(self._next(), shape, jnp.bfloat16, lo, hi)
    def permutation(self, n):
        return jax.random.permutation(self._next(), n)


kernel_name = 'recurrent_scan__sliding_block__dense_activation_mish__prompt'

def setup_inputs():
    _rng = _Rng(jax.random.key(int.from_bytes(__import__("os").urandom(4), "little")))
    _w = (lambda a: (lambda t: t.astype(jnp.bfloat16) if jnp.issubdtype(t.dtype, jnp.floating) else t)(jnp.asarray(a)))
    def _A_setup():
        B, S, D = 1, 2048, 576
        return {
            "x": _w((lambda *s: _rng.normal(s) * 0.05)(B, S, D)),
            "wqkv": _w((lambda *s: _rng.normal(s) * 0.1)(D, 3 * D)),
            "wo": _w((lambda *s: _rng.normal(s) * 0.1)(D, D)),
        }
    _A_in = _A_setup()

    def _B_setup():
        B, S, D, F = 1, 2048, 576, 4608
        return {
            "x": _w((lambda *s: _rng.normal(s) * 0.05)(B, S, D)),
            "w1": _w((lambda *s: _rng.normal(s) * 0.05)(D, F) * (D ** -0.5)),
            "b1": _w((lambda *s: _rng.normal(s) * 0.05)(F)),
            "w2": _w((lambda *s: _rng.normal(s) * 0.05)(F, D) * (F ** -0.5)),
        }
    _B_in = _B_setup()

    return {
        "A_x": _A_in["x"],
        "A_wqkv": _A_in["wqkv"],
        "A_wo": _A_in["wo"],
        "B_x": _B_in["x"],
        "B_w1": _B_in["w1"],
        "B_b1": _B_in["b1"],
        "B_w2": _B_in["w2"],
    }

def reference(A_x, A_wqkv, A_wo, B_x, B_w1, B_b1, B_w2):
    def _A_ref(x, wqkv, wo):
        B, S, D = x.shape
        H = 32; Dh = D // H; W = 256
        qkv = (lambda x, *d: x.transpose(*d))((x @ wqkv).reshape(B, S, 3, H, Dh), 2, 0, 3, 1, 4)
        q, k, v = qkv[0], qkv[1], qkv[2]
        scores = jnp.einsum("bhqd,bhkd->bhqk", q, k) * (Dh ** -0.5)
        idx = jnp.arange(S)
        mask = (idx[:, None] - idx[None, :] >= 0) & (idx[:, None] - idx[None, :] < W)
        scores = jnp.where(mask[None, None], scores, -1e9)
        p = _softmax(scores, axis=-1)
        o = jnp.einsum("bhqk,bhkd->bhqd", p, v)
        return (lambda x, *d: x.transpose(*d))(o, 0, 2, 1, 3).reshape(B, S, D) @ wo

    def _B_ref(x, w1, b1, w2):
        h = jnp.einsum("bsd,df->bsf", x, w1) + b1
        sp = jnp.log1p(jnp.exp(-jnp.abs(h))) + jnp.where(h > 0, h, jnp.zeros_like(h))
        act = h * jnp.tanh(sp)
        return jnp.einsum("bsf,fd->bsd", act, w2)

    x = A_x
    xn = _layernorm(x, axis=-1)
    s = _A_ref(xn, A_wqkv, A_wo)
    g = _silu(_B_ref(xn, B_w1, B_b1, B_w2))
    return x + s * g
```

```python
import jax
import jax.numpy as jnp
import numpy as np
from jax import lax
import jax.experimental.pallas as pl
import jax.experimental.pallas.tpu as pltpu

S, D, F = 2048, 576, 4608
H, DH, W = 32, 18, 256
DP = 640
NS = 256
FC = 512
NC = F // FC
G = 8
GH = H // G
GD = GH * DH
BQ = 128
LOG2E = 1.4426950408889634
NT = (((1,), (1,)), ((), ()))
f32, bf16 = jnp.float32, jnp.bfloat16


def _kernel(x_ref, wqkv_ref, wo_ref, w1_ref, b1_ref, w2_ref, o_ref,
            w1t, w2t, wvt, wot, kw, qw, vt, xnt, ot, acc):
    step = pl.program_id(0)

    @pl.when(step == 0)
    def _prep():
        row = lax.broadcasted_iota(jnp.int32, (DP - D, FC), 0)
        for c in range(NC):
            sl = slice(c * FC, (c + 1) * FC)
            tail = jnp.where(row == 0, b1_ref[:, sl].astype(f32), 0.0).astype(bf16)
            w1t[c] = jnp.concatenate([w1_ref[:, sl], tail], axis=0).T
            w2c = jnp.concatenate([w2_ref[sl, :], jnp.zeros((FC, DP - D), bf16)], axis=1)
            w2t[c] = w2c.T[:D]
        zc = jnp.zeros((D, DP - D), bf16)
        wvt[...] = jnp.concatenate([wqkv_ref[:, 2 * D:], zc], axis=1).T[:D]
        wot[...] = jnp.concatenate([wo_ref[...], zc], axis=1).T[:D]
        lane = lax.broadcasted_iota(jnp.int32, (W, 128), 1)
        kpad = jnp.where(lane == 127, -1e30, 0.0).astype(bf16)
        for g in range(G):
            kw[g, 0:W, :] = kpad
        vt[:, :, 0:W] = jnp.zeros((H, 32, W), bf16)

    x = x_ref[...].astype(f32)
    mu = jnp.mean(x, axis=-1, keepdims=True)
    xc = x - mu
    var = jnp.mean(xc * xc, axis=-1, keepdims=True)
    xn = (xc * lax.rsqrt(var + 1e-5)).astype(bf16)
    lane = lax.broadcasted_iota(jnp.int32, (NS, DP - D), 1)
    one = jnp.where(lane == 0, 1.0, 0.0).astype(bf16)
    xnt[...] = jnp.concatenate([xn, one], axis=1).T

    r0 = pl.multiple_of(step * NS, NS)
    qk = jnp.dot(xn, wqkv_ref[:, :2 * D], preferred_element_type=f32)
    lane = lax.broadcasted_iota(jnp.int32, (NS, 128), 1)
    qkp = jnp.concatenate([qk, jnp.zeros((NS, 128), f32)], axis=1)
    for g in range(G):
        qg = qkp[:, g * GD:g * GD + 128] * (DH ** -0.5 * LOG2E)
        qw[g] = jnp.where(lane == 127, 1.0, qg).astype(bf16)
        kg = qkp[:, D + g * GD:D + g * GD + 128]
        kw[g, pl.ds(r0 + W, NS), :] = jnp.where(lane < GD, kg, 0.0).astype(bf16)
    v = jnp.dot(wvt[...], xnt[0:D, :], preferred_element_type=f32)
    row = lax.broadcasted_iota(jnp.int32, (32, NS), 0)
    vp = jnp.concatenate([v, jnp.zeros((32, NS), f32)], axis=0)
    for h in range(H):
        vh = vp[h * DH:h * DH + 32]
        vh = jnp.where(row < DH, vh, jnp.where(row == DH, 1.0, 0.0))
        vt[h, :, pl.ds(r0 + W, NS)] = vh.astype(bf16)

    def ffn(c):
        h = jnp.dot(w1t[c], xnt[...], preferred_element_type=f32)
        e = jnp.exp(jnp.minimum(h, 20.0))
        n = e * (e + 2.0)
        act = h * n * pl.reciprocal(n + 2.0, approx=True)
        return jnp.dot(w2t[c], act.astype(bf16), preferred_element_type=f32)

    def attn(g):
        r = lax.broadcasted_iota(jnp.int32, (BQ, BQ), 0)
        cidx = lax.broadcasted_iota(jnp.int32, (BQ, BQ), 1)
        upper = r > cidx
        for b in range(NS // BQ):
            q0 = pl.multiple_of(r0 + b * BQ, BQ)
            kwin = kw[g, pl.ds(q0, 3 * BQ), :]
            qb = qw[g, b * BQ:(b + 1) * BQ, :].astype(f32)
            for i in range(GH):
                keep = ((cidx >= i * DH) & (cidx < (i + 1) * DH)) | (cidx == 127)
                qm = jnp.where(keep, qb, 0.0).astype(bf16)
                st = lax.dot_general(kwin, qm, NT, preferred_element_type=f32)
                mid = st[BQ:2 * BQ]
                mer = jnp.where(upper, st[:BQ], st[2 * BQ:])
                m = jnp.max(jnp.maximum(mer, mid), axis=0, keepdims=True)
                p1 = jnp.exp2(mer - m)
                p2 = jnp.exp2(mid - m)
                p = jnp.concatenate([jnp.where(upper, p1, 0.0), p2,
                                     jnp.where(upper, 0.0, p1)], axis=0).astype(bf16)
                o = jnp.dot(vt[g * GH + i, :, pl.ds(q0, 3 * BQ)], p,
                            preferred_element_type=f32)
                on = o[0:DH] / o[DH:DH + 1]
                ot[g, i * DH:(i + 1) * DH, b * BQ:(b + 1) * BQ] = on

    acc[...] = ffn(NC - 1)

    def body(c, carry):
        attn(c)
        acc[...] += ffn(c)
        return carry
    lax.fori_loop(0, G, body, 0)

    s = jnp.dot(wot[...], ot[...].reshape(D, NS).astype(bf16), preferred_element_type=f32)
    a = acc[...]
    y = s * a / (1.0 + jnp.exp(-a))
    yt = jnp.concatenate([y, jnp.zeros((DP - D, NS), f32)], axis=0).T
    o_ref[...] = (x + yt[:, :D]).astype(o_ref.dtype)


@jax.jit
def pallas_recurrent_scan__sliding_block__dense_activation_mish__prompt_kernel(
    A_x, A_wqkv, A_wo, B_x, B_w1, B_b1, B_w2,
):
    full = lambda shape: pl.BlockSpec(shape, lambda i: (0,) * len(shape),
                                      pipeline_mode=pl.Buffered(1))
    out = pl.pallas_call(
        _kernel,
        grid=(S // NS,),
        in_specs=[pl.BlockSpec((NS, D), lambda i: (i, 0)),
                  full((D, 3 * D)), full((D, D)), full((D, F)), full((1, F)), full((F, D))],
        out_specs=pl.BlockSpec((NS, D), lambda i: (i, 0)),
        out_shape=jax.ShapeDtypeStruct((S, D), A_x.dtype),
        scratch_shapes=[
            pltpu.VMEM((NC, FC, DP), bf16),
            pltpu.VMEM((NC, D, FC), bf16),
            pltpu.VMEM((D, D), bf16),
            pltpu.VMEM((D, D), bf16),
            pltpu.VMEM((G, S + W, 128), bf16),
            pltpu.VMEM((G, NS, 128), bf16),
            pltpu.VMEM((H, 32, S + W), bf16),
            pltpu.VMEM((DP, NS), bf16),
            pltpu.VMEM((G, GD, NS), f32),
            pltpu.VMEM((D, NS), f32),
        ],
        compiler_params=pltpu.CompilerParams(
            dimension_semantics=("arbitrary",), vmem_limit_bytes=100 << 20),
    )(A_x.reshape(S, D), A_wqkv, A_wo, B_w1, B_b1.reshape(1, F), B_w2)
    return out.reshape(1, S, D)
```

```python
import jax
import jax.numpy as jnp
import numpy as np
from jax import lax
import jax.experimental.pallas as pl
import jax.experimental.pallas.tpu as pltpu

S, D, F = 2048, 576, 4608
H, DH, W = 32, 18, 256
DP = 640
NS = 512
FC = 512
NB = S // NS
NC = F // FC
G = 8
GH = H // G
GD = GH * DH
BQ = 128
LOG2E = 1.4426950408889634
NT = (((1,), (1,)), ((), ()))
f32, bf16 = jnp.float32, jnp.bfloat16


def pk(v):
    return pltpu.bitcast(v, jnp.int32)


def upk(v):
    return pltpu.bitcast(v, bf16)


def _kernel(x_hbm, wqkv_hbm, wo_hbm, w1_hbm, b1_ref, w2_hbm, o_ref,
            wqkv_ref, wo_ref, w1_ref, w2_ref, sems,
            x_ref, w1a, w1b, wvt, wot, kw, qw, vt, xnt, ot, acc):
    step = pl.program_id(0)

    def w1_copy(c):
        return pltpu.make_async_copy(w1_hbm.at[:, pl.ds(c * FC, FC)], w1_ref.at[c], sems.at[c])

    def w2_copy(c):
        return pltpu.make_async_copy(w2_hbm.at[:, pl.ds(c * FC, FC)], w2_ref.at[c], sems.at[NC + c])

    qkv_copy = pltpu.make_async_copy(wqkv_hbm, wqkv_ref, sems.at[2 * NC])
    wo_copy = pltpu.make_async_copy(wo_hbm, wo_ref, sems.at[2 * NC + 1])

    def x_copy(i):
        return pltpu.make_async_copy(x_hbm.at[:, pl.ds(pl.multiple_of(i * NS, NS), NS)],
                                     x_ref.at[i], sems.at[2 * NC + 2 + i])

    def transpose_w1(c, w1t):
        row = lax.broadcasted_iota(jnp.int32, (DP - D, FC), 0)
        tail = jnp.where(row == 0, b1_ref[c].astype(f32), 0.0).astype(bf16)
        w1t[...] = pk(jnp.concatenate([w1_ref[c], tail], axis=0).T)

    def fetch_chunk(c):
        @pl.when(step == 0)
        def _():
            w1_copy(c + 1).wait()
            w2_copy(c).wait()

    zc = jnp.zeros((D, DP - D), bf16)

    @pl.when(step == 0)
    def _prep():
        x_copy(0).start()
        qkv_copy.start()
        lane = lax.broadcasted_iota(jnp.int32, (W, 128), 1)
        kpad = jnp.where(lane == 127, -1e30, 0.0).astype(bf16)
        for g in range(G):
            kw[g, 0:W // 2, :] = pk(kpad)
        vt[:, :, 0:W] = jnp.zeros((H, 16, W), jnp.int32)
        acc[...] = jnp.zeros((D, NS), f32)
        x_copy(0).wait()
        qkv_copy.wait()
        for c in range(NC):
            w1_copy(c).start()
            w2_copy(c).start()
        wo_copy.start()
        for i in range(1, NB):
            x_copy(i).start()
        wvt[...] = pk(jnp.concatenate([wqkv_ref[:, 2 * D:], zc], axis=1).T[:D])

    def head(i):
        x = x_ref[i].astype(f32)
        mu = jnp.mean(x, axis=0, keepdims=True)
        xc = x - mu
        var = jnp.mean(xc * xc, axis=0, keepdims=True)
        xn = (xc * lax.rsqrt(var + 1e-5)).astype(bf16)
        row = lax.broadcasted_iota(jnp.int32, (DP - D, NS), 0)
        one = jnp.where(row == 0, 1.0, 0.0).astype(bf16)
        xnp = jnp.concatenate([xn, one], axis=0)
        xnt[...] = pk(xnp)
        xn = xnp.T[:, :D]

        r0 = pl.multiple_of(i * NS, NS)
        qk = jnp.dot(xn, wqkv_ref[:, :2 * D], preferred_element_type=f32)
        lane = lax.broadcasted_iota(jnp.int32, (NS, 128), 1)
        qkp = jnp.concatenate([qk, jnp.zeros((NS, 128), f32)], axis=1)
        for g in range(G):
            qg = qkp[:, g * GD:g * GD + 128] * (DH ** -0.5 * LOG2E)
            qw[g] = jnp.where(lane == 127, 1.0, qg)
            kg = qkp[:, D + g * GD:D + g * GD + 128]
            kw[g, pl.ds(pl.multiple_of(i * (NS // 2) + W // 2, 64), NS // 2), :] = pk(
                jnp.where(lane < GD, kg, 0.0).astype(bf16))
        v = jnp.dot(upk(wvt[...]), upk(xnt[0:D // 2, :]), preferred_element_type=f32)
        row = lax.broadcasted_iota(jnp.int32, (32, NS), 0)
        vp = jnp.concatenate([v, jnp.zeros((32, NS), f32)], axis=0)
        for h in range(H):
            vh = vp[h * DH:h * DH + 32]
            vh = jnp.where(row < DH, vh, jnp.where(row == DH, 1.0, 0.0))
            vt[h, :, pl.ds(r0 + W, NS)] = pk(vh.astype(bf16))


    @pl.when(step == 0)
    def _():
        head(0)
        w1_copy(0).wait()
        transpose_w1(0, w1a)

    r0 = pl.multiple_of(step * NS, NS)

    def ffn1(w1t):
        return jnp.dot(upk(w1t[...]), upk(xnt[...]), preferred_element_type=f32)

    def mish(h):
        e = jnp.exp(jnp.minimum(h, 20.0))
        n = e * (e + 2.0)
        return (h * n * pl.reciprocal(n + 2.0, approx=True)).astype(bf16)

    def ffn2(c, act):
        return jnp.dot(w2_ref[c], act,
                       preferred_element_type=f32)

    r = lax.broadcasted_iota(jnp.int32, (BQ, BQ), 0)
    cidx = lax.broadcasted_iota(jnp.int32, (BQ, BQ), 1)
    upper = r > cidx
    tiles = [(b, i) for b in range(NS // BQ) for i in range(GH)]

    def scores(g, b, i):
        q0 = pl.multiple_of(step * (NS // 2) + b * (BQ // 2), BQ // 2)
        kwin = upk(kw[g, pl.ds(q0, 3 * BQ // 2), :])
        qb = qw[g, b * BQ:(b + 1) * BQ, :]
        keep = ((cidx >= i * DH) & (cidx < (i + 1) * DH)) | (cidx == 127)
        qm = jnp.where(keep, qb, 0.0).astype(bf16)
        return lax.dot_general(kwin, qm, NT, preferred_element_type=f32)

    def softmax(st):
        mid = st[BQ:2 * BQ]
        mer = jnp.where(upper, st[:BQ], st[2 * BQ:])
        m = jnp.max(jnp.maximum(mer, mid), axis=0, keepdims=True)
        p1 = jnp.exp2(mer - m)
        p2 = jnp.exp2(mid - m)
        return jnp.concatenate([jnp.where(upper, p1, 0.0), p2,
                                jnp.where(upper, 0.0, p1)], axis=0).astype(bf16)

    def pv(g, b, i, p):
        q0 = pl.multiple_of(r0 + b * BQ, BQ)
        o = jnp.dot(upk(vt[g * GH + i, :, pl.ds(q0, 3 * BQ)]), p, preferred_element_type=f32)
        on = o[0:24] * pl.reciprocal(o[DH:DH + 1], approx=True)
        ot[g, i * DH:(i + 1) * DH, b * BQ:(b + 1) * BQ] = on[0:DH]


    def part(c, cur, nxt):
        transpose_w1(c + 1, nxt)
        sts, hs = [], []
        for n in range(NS // BQ):
            sts += [scores(c, n, i) for i in range(GH)]
            hs.append(jnp.dot(upk(cur[...]), upk(xnt[:, n * BQ:(n + 1) * BQ]), preferred_element_type=f32))
        h = jnp.concatenate(hs, axis=1)
        ps = [softmax(st) for st in sts]
        act = mish(h)
        for (b, i), p in zip(tiles, ps):
            pv(c, b, i, p)
        acc[...] += ffn2(c, act)

    def body(j, carry):
        fetch_chunk(2 * j)
        fetch_chunk(2 * j + 1)
        part(2 * j, w1a, w1b)
        part(2 * j + 1, w1b, w1a)
        return carry
    lax.fori_loop(0, G // 2, body, 0)


    @pl.when(step == 0)
    def _():
        w2_copy(NC - 1).wait()
        wo_copy.wait()
        wot[...] = pk(jnp.concatenate([wo_ref[...], zc], axis=1).T[:D])

    def tail():
        s = jnp.dot(upk(wot[...]), ot[...].reshape(D, NS).astype(bf16), preferred_element_type=f32)
        a = acc[...] + ffn2(NC - 1, mish(ffn1(w1a)))
        acc[...] = jnp.zeros((D, NS), f32)
        y = s * a * pl.reciprocal(1.0 + jnp.exp(-a), approx=True)
        o_ref[...] = (x_ref[step].astype(f32) + y).astype(o_ref.dtype)

    @pl.when(step < NB - 1)
    def _():
        x_copy(step + 1).wait()
        tail()
        transpose_w1(0, w1a)
        head(step + 1)

    pl.when(step == NB - 1)(tail)


@jax.jit
def pallas_recurrent_scan__sliding_block__dense_activation_mish__prompt_kernel(
    A_x, A_wqkv, A_wo, B_x, B_w1, B_b1, B_w2,
):
    full = lambda shape: pl.BlockSpec(shape, lambda i: (0,) * len(shape),
                                      pipeline_mode=pl.Buffered(1))
    hbm = pl.BlockSpec(memory_space=pltpu.HBM)
    out = pl.pallas_call(
        _kernel,
        grid=(S // NS,),
        in_specs=[hbm,
                  hbm, hbm, hbm, full((NC, 1, FC)), hbm],
        out_specs=pl.BlockSpec((D, NS), lambda i: (0, i)),
        out_shape=jax.ShapeDtypeStruct((D, S), A_x.dtype),
        scratch_shapes=[
            pltpu.VMEM((D, 3 * D), bf16),
            pltpu.VMEM((D, D), bf16),
            pltpu.VMEM((NC, D, FC), bf16),
            pltpu.VMEM((NC, D, FC), bf16),
            pltpu.SemaphoreType.DMA((2 * NC + 2 + NB,)),
            pltpu.VMEM((NB, D, NS), bf16),
            pltpu.VMEM((FC // 2, DP), jnp.int32),
            pltpu.VMEM((FC // 2, DP), jnp.int32),
            pltpu.VMEM((D // 2, D), jnp.int32),
            pltpu.VMEM((D // 2, D), jnp.int32),
            pltpu.VMEM((G, (S + W) // 2, 128), jnp.int32),
            pltpu.VMEM((G, NS, 128), f32),
            pltpu.VMEM((H, 16, S + W), jnp.int32),
            pltpu.VMEM((DP // 2, NS), jnp.int32),
            pltpu.VMEM((G, GD, NS), f32),
            pltpu.VMEM((D, NS), f32),
        ],
        compiler_params=pltpu.CompilerParams(
            dimension_semantics=("arbitrary",), vmem_limit_bytes=100 << 20),
    )(A_x.reshape(S, D).T, A_wqkv, A_wo, B_w1, B_b1.reshape(NC, 1, FC), B_w2.T)
    return out.T.reshape(1, S, D)
```
